```python
import jax
import jax.numpy as jnp

def _softmax(x, axis=-1):
    return jax.nn.softmax(x, axis=axis)

def _gelu(x):
    return jax.nn.gelu(x, approximate=True)

def _silu(x):
    return jax.nn.silu(x)

def _sigmoid(x):
    return jax.nn.sigmoid(x)

def _layernorm(x, axis=-1, eps=1e-05):
    m = jnp.mean(x, axis=axis, keepdims=True)
    v = jnp.var(x, axis=axis, keepdims=True)
    return (x - m) / jnp.sqrt(v + eps)

def _scatter_add(tgt, idx, src, axis=0):
    return tgt.at[idx].add(src)

def _segment_sum(src, seg, n):
    return jax.ops.segment_sum(src, seg, n)

class _Rng:

    def __init__(self, key):
        self._k = key

    def _next(self):
        self._k, sub = jax.random.split(self._k)
        return sub

    def normal(self, shape):
        return jax.random.normal(self._next(), shape, dtype=jnp.bfloat16)

    def randint(self, lo, hi, shape):
        return jax.random.randint(self._next(), shape, lo, hi, dtype=jnp.int32)

    def uniform(self, shape, lo=0.0, hi=1.0):
        return jax.random.uniform(self._next(), shape, jnp.bfloat16, lo, hi)

    def permutation(self, n):
        return jax.random.permutation(self._next(), n)
kernel_name = 'adaLN_cond__gqa_block_cached__moe_arch_mod__decode'

def setup_inputs():
    _rng = _Rng(jax.random.key(int.from_bytes(__import__("os").urandom(4), "little")))
    _w = lambda a: (lambda t: t.astype(jnp.bfloat16) if jnp.issubdtype(t.dtype, jnp.floating) else t)(jnp.asarray(a))

    def _A_setup():
        B, Sq, D = (4, 1, 512)
        Hq, Hkv, Sk, Dh = (32, 32, 8192, 128)
        assert Hq % Hkv == 0, (Hq, Hkv)
        return {'x': _w((lambda *s: _rng.normal(s) * 0.05)(B, Sq, D)), 'k_cache': _w((lambda *s: _rng.normal(s) * 0.05)(B, Hkv, Sk, Dh)), 'v_cache': _w((lambda *s: _rng.normal(s) * 0.05)(B, Hkv, Sk, Dh)), 'wq': _w((lambda *s: _rng.normal(s) * 0.05)(D, Hq * Dh) * D ** (-0.5)), 'wo': _w((lambda *s: _rng.normal(s) * 0.05)(Hq * Dh, D) * (Hq * Dh) ** (-0.5))}
    _A_in = _A_setup()

    def _B_setup():
        B, S, D, F, C = (4, 1, 512, 1376, 1)
        return {'x': _w((lambda *s: _rng.normal(s) * 0.05)(B, S, D)), 'w_r': _w((lambda *s: _rng.normal(s) * 0.05)(D)), 'w_gate': _w((lambda *s: _rng.normal(s) * 0.05)(D, F)), 'w_up': _w((lambda *s: _rng.normal(s) * 0.05)(D, F)), 'w_down': _w((lambda *s: _rng.normal(s) * 0.05)(F, D))}
    _B_in = _B_setup()
    return {'A_x': _A_in['x'], 'A_k_cache': _A_in['k_cache'], 'A_v_cache': _A_in['v_cache'], 'A_wq': _A_in['wq'], 'A_wo': _A_in['wo'], 'B_x': _B_in['x'], 'B_w_r': _B_in['w_r'], 'B_w_gate': _B_in['w_gate'], 'B_w_up': _B_in['w_up'], 'B_w_down': _B_in['w_down'], 'c': _w((lambda *s: _rng.normal(s) * 0.05)(4, 512)), 'w_mod': _w((lambda *s: _rng.normal(s) * 0.05)(512, 6 * 512) * 512 ** (-0.5))}

def reference(A_x, A_k_cache, A_v_cache, A_wq, A_wo, B_x, B_w_r, B_w_gate, B_w_up, B_w_down, c, w_mod):

    def _A_ref(x, k_cache, v_cache, wq, wo):
        B, Sq, D = x.shape
        Hq, Dh = (32, 128)
        Hkv = k_cache.shape[1]
        rep = Hq // Hkv
        q = (lambda x, *d: x.transpose(*d))((x @ wq).reshape(B, Sq, Hq, Dh), 0, 2, 1, 3)
        k = jnp.repeat(k_cache, rep, axis=1)
        v = jnp.repeat(v_cache, rep, axis=1)
        scores = jnp.einsum('bhqd,bhkd->bhqk', q, k) * Dh ** (-0.5)
        p = _softmax(scores, axis=-1)
        o = jnp.einsum('bhqk,bhkd->bhqd', p, v)
        return (lambda x, *d: x.transpose(*d))(o, 0, 2, 1, 3).reshape(B, Sq, Hq * Dh) @ wo

    def _B_ref(x, w_r, w_gate, w_up, w_down):
        B, S, D = x.shape
        C = 1
        r = x @ w_r
        idx = jnp.argsort(-r, axis=-1)[:, :C]
        idx_e = jnp.repeat(idx.reshape(B, C, 1), D, axis=2)
        x_sel = jnp.take_along_axis(x, idx_e, axis=1)
        g = _silu(x_sel @ w_gate)
        u = x_sel @ w_up
        y = g * u @ w_down
        r_sel = _sigmoid(jnp.take_along_axis(r, idx, axis=1))
        y = y * r_sel.reshape(B, C, 1)
        b_off = (jnp.arange(B) * S).reshape(B, 1)
        flat_idx = (idx + b_off).reshape(B * C)
        zero = (x * 0.0).reshape(B * S, D)
        upd = _scatter_add(zero, flat_idx, y.reshape(B * C, D), axis=0)
        return x + upd.reshape(B, S, D)
    x = A_x
    mod = (_silu(c) @ w_mod).reshape(c.shape[0], 6, 1, -1)
    sa, ca, ga, sb, cb, gb = (mod[:, 0].copy(), mod[:, 1].copy(), mod[:, 2].copy(), mod[:, 3].copy(), mod[:, 4].copy(), mod[:, 5].copy())
    h = _layernorm(x, axis=-1) * (1 + ca) + sa
    x = x + ga * _A_ref(h, A_k_cache, A_v_cache, A_wq, A_wo)
    h = _layernorm(x, axis=-1) * (1 + cb) + sb
    x = x + gb * _B_ref(h, B_w_r, B_w_gate, B_w_up, B_w_down)
    return x
```

```python
import functools

import jax
import jax.numpy as jnp
import jax.experimental.pallas as pl
import jax.experimental.pallas.tpu as pltpu

_B, _D = 4, 512
_H, _DH = 32, 128
_EPS = 1e-5


def _layernorm(x):
    m = jnp.mean(x, axis=-1, keepdims=True)
    xc = x - m
    v = jnp.mean(xc * xc, axis=-1, keepdims=True)
    return xc / jnp.sqrt(v + _EPS)


def _dot(a, b):
    return jnp.dot(a, b, preferred_element_type=jnp.float32)


def _dot_nt(a, b):
    return jax.lax.dot_general(a, b, (((1,), (1,)), ((), ())),
                               preferred_element_type=jnp.float32)


def _kernel(x_hbm, c_hbm, wr_hbm, wmod_hbm, wq_hbm, wo_hbm, wg_hbm, wu_hbm, wd_hbm,
            k_hbm, v_hbm, o_ref,
            x_v, c_v, wr_v, wmod_v, wq_v, wo_v, wg_v, wu_v, wd_v, kbuf, vbuf, q_s,
            wsem, ksem, vsem, *, nbuf, grp, rows, streams, sk, roll, nocompute, wdrows, wdsplit, early):
    f32, bf16 = jnp.float32, jnp.bfloat16
    n_blocks = _B * _H // grp
    blk_rows = grp * sk
    n_chunks = blk_rows // rows
    per_stream = n_chunks // streams
    assert per_stream * streams == n_chunks and per_stream % roll == 0

    def copy(src, dst, sem, prio):
        pltpu.make_async_copy(src, dst, sem).start(priority=prio)

    def wait_all(buf, sem):
        pltpu.make_async_copy(buf, buf, sem).wait()

    def start_block(i, slot, lo=0, hi=None):
        hi = per_stream // roll if hi is None else hi
        base = pl.multiple_of(i * blk_rows, blk_rows)

        def body(t, carry):
            for u in range(roll):
                for st in range(streams):
                    off = pl.multiple_of((st * per_stream + t * roll + u) * rows, rows)
                    copy(k_hbm.at[pl.ds(base + off, rows)], kbuf.at[slot, pl.ds(off, rows)], ksem.at[slot], 0)
                    copy(v_hbm.at[pl.ds(base + off, rows)], vbuf.at[slot, pl.ds(off, rows)], vsem.at[slot], 1)
            return carry
        jax.lax.fori_loop(lo, hi, body, 0)

    def start_rows(pairs, n, unroll):
        def body(t, carry):
            for src, dst, sem, rr, first, prio in pairs:
                sl = pl.ds(pl.multiple_of((first + t) * rr, rr), rr)
                copy(src.at[sl], dst.at[sl], sem, prio)
            return carry
        jax.lax.fori_loop(0, n, body, 0, unroll=unroll)

    ff = wg_hbm.shape[0]

    def start_gate_up():
        start_rows([(wg_hbm, wg_v, wsem.at[6], 32, 0, 0), (wu_hbm, wu_v, wsem.at[7], 32, 0, 1)], ff // 32, 1)

    wd_edges = [ff * j // wdsplit // wdrows * wdrows for j in range(wdsplit)] + [ff]

    def start_down():
        nch = ff // wdrows
        assert nch * wdrows == ff
        for j in range(wdsplit):
            c0, c1 = wd_edges[j] // wdrows, wd_edges[j + 1] // wdrows
            half = (c1 - c0) // 2
            start_rows([(wd_hbm, wd_v, wsem.at[8 + j], wdrows, c0, 0),
                        (wd_hbm, wd_v, wsem.at[8 + j], wdrows, c0 + half, 1)], half, 1)
            if (c1 - c0) % 2:
                sl = pl.ds((c1 - 1) * wdrows, wdrows)
                copy(wd_hbm.at[sl], wd_v.at[sl], wsem.at[8 + j], 0)

    copy(c_hbm, c_v, wsem.at[0], 0)
    copy(x_hbm, x_v, wsem.at[1], 1)
    start_rows([(wmod_hbm, wmod_v, wsem.at[3], 16, 0, 0), (wq_hbm, wq_v, wsem.at[4], 16, 0, 1)], 32, 4)
    copy(wr_hbm, wr_v, wsem.at[2], 1)
    start_rows([(wo_hbm, wo_v, wsem.at[5], 32, 0, 0), (wo_hbm, wo_v, wsem.at[5], 32, 64, 1)], 64, 4)
    if early:
        start_block(0, 0, 0, early)

    wait_all(c_v, wsem.at[0])
    wait_all(x_v, wsem.at[1])
    cc = c_v[...].astype(f32)
    sc = (cc * jax.nn.sigmoid(cc)).astype(bf16)
    x = x_v[...].astype(f32)
    ln_x = _layernorm(x)
    wait_all(wmod_v, wsem.at[3])
    mod = _dot(sc, wmod_v[...])
    sa, ca, ga, sb, cb, gb = (mod[:, j * _D:(j + 1) * _D] for j in range(6))
    h = (ln_x * (1.0 + ca) + sa).astype(bf16)
    wait_all(wq_v, wsem.at[4])
    q = _dot(h, wq_v[...]).astype(bf16)
    for hh in range(_H):
        q_s[hh] = q[:, hh * _DH:(hh + 1) * _DH]

    start_block(0, 0, early, None)
    for j in range(1, nbuf):
        start_block(j, j)
    wait_all(wo_v, wsem.at[5])

    scale = _DH ** (-0.5)
    row = jax.lax.broadcasted_iota(jnp.int32, (_B, _DH), 0)

    def step(i, acc):
        slot = i % nbuf
        b = (i * grp) // _H
        h0 = (i * grp) % _H
        wait_all(kbuf.at[slot], ksem.at[slot])
        ps, ls = [], []
        if not nocompute:
            for g in range(grp):
                s = _dot_nt(q_s[h0 + g], kbuf[slot, pl.ds(g * sk, sk), :]) * scale
                m = jnp.max(s, axis=-1, keepdims=True)
                p = jnp.exp(s - m)
                ls.append(jnp.sum(p, axis=-1, keepdims=True))
                ps.append(p.astype(bf16))

        @pl.when(i == n_blocks - 1)
        def _():
            start_down()

        wait_all(vbuf.at[slot], vsem.at[slot])
        os_ = []
        if not nocompute:
            for g in range(grp):
                o = _dot(ps[g], vbuf[slot, pl.ds(g * sk, sk), :]) / ls[g]
                os_.append(jnp.where(row == b, o, 0.0).astype(bf16))

        @pl.when(i + nbuf < n_blocks)
        def _():
            start_block(i + nbuf, slot)

        @pl.when(i == n_blocks - 2)
        def _():
            start_gate_up()

        if nocompute:
            return acc
        o_cat = jnp.concatenate(os_, axis=-1) if grp > 1 else os_[0]
        wo_h = wo_v[pl.ds(pl.multiple_of(h0 * _DH, grp * _DH), grp * _DH), :]
        return acc + _dot(o_cat, wo_h)

    attn = jax.lax.fori_loop(0, n_blocks, step, jnp.zeros((_B, _D), f32))

    x1 = x + ga * attn
    h2 = _layernorm(x1) * (1.0 + cb) + sb
    h2b = h2.astype(bf16)
    wait_all(wr_v, wsem.at[2])
    wr = wr_v[...].astype(f32)
    r = sum(h2[:, j * 128:(j + 1) * 128] * wr[j:j + 1, :] for j in range(_D // 128))
    r = jnp.sum(r, axis=-1, keepdims=True)
    wait_all(wg_v, wsem.at[6])
    g = _dot_nt(h2b, wg_v[...])
    g = g * jax.nn.sigmoid(g)
    wait_all(wu_v, wsem.at[7])
    u = _dot_nt(h2b, wu_v[...])
    a = (g * u).astype(bf16)
    y = None
    for j in range(wdsplit):
        lo, hi = wd_edges[j], wd_edges[j + 1]
        wait_all(wd_v.at[pl.ds(lo, hi - lo)], wsem.at[8 + j])
        part = _dot(a[:, lo:hi], wd_v[lo:hi, :])
        y = part if y is None else y + part
    y = y * jax.nn.sigmoid(r)
    upd = h2 * 0.0 + y
    o_ref[...] = (x1 + gb * (h2 + upd)).astype(o_ref.dtype)


def _build(A_x, A_k_cache, A_v_cache, A_wq, A_wo, B_w_r, B_w_gate, B_w_up, B_w_down,
           c, w_mod, *, nbuf=2, grp=2, rows=128, streams=4, roll=2, nocompute=False, wdrows=32, wdsplit=1, early=0):
    bf16 = jnp.bfloat16
    sk = A_k_cache.shape[2]
    ff = B_w_gate.shape[1]
    hbm = pl.BlockSpec(memory_space=pltpu.HBM)
    out = pl.pallas_call(
        functools.partial(_kernel, nbuf=nbuf, grp=grp, rows=rows, streams=streams, sk=sk, roll=roll,
                          nocompute=nocompute, wdrows=wdrows, wdsplit=wdsplit, early=early),
        out_shape=jax.ShapeDtypeStruct((_B, _D), A_x.dtype),
        in_specs=[hbm] * 11,
        out_specs=pl.BlockSpec(memory_space=pltpu.VMEM),
        scratch_shapes=[
            pltpu.VMEM((_B, _D), bf16),
            pltpu.VMEM((_B, _D), bf16),
            pltpu.VMEM((_D // 128, 128), bf16),
            pltpu.VMEM((_D, 6 * _D), bf16),
            pltpu.VMEM((_D, _H * _DH), bf16),
            pltpu.VMEM((_H * _DH, _D), bf16),
            pltpu.VMEM((ff, _D), bf16),
            pltpu.VMEM((ff, _D), bf16),
            pltpu.VMEM((ff, _D), bf16),
            pltpu.VMEM((nbuf, grp * sk, _DH), bf16),
            pltpu.VMEM((nbuf, grp * sk, _DH), bf16),
            pltpu.VMEM((_H, _B, _DH), bf16),
            pltpu.SemaphoreType.DMA((8 + wdsplit,)),
            pltpu.SemaphoreType.DMA((nbuf,)),
            pltpu.SemaphoreType.DMA((nbuf,)),
        ],
        compiler_params=pltpu.CompilerParams(vmem_limit_bytes=100 * 1024 * 1024),
        name="adaln_gqa_mod_decode",
    )(A_x.reshape(_B, _D), c, B_w_r.reshape(_D // 128, 128), w_mod, A_wq, A_wo,
      B_w_gate.T, B_w_up.T, B_w_down,
      A_k_cache.reshape(-1, _DH), A_v_cache.reshape(-1, _DH))
    return out.reshape(A_x.shape)


@jax.jit
def pallas_adaLN_cond__gqa_block_cached__moe_arch_mod__decode_kernel(
    A_x: jax.Array,
    A_k_cache: jax.Array,
    A_v_cache: jax.Array,
    A_wq: jax.Array,
    A_wo: jax.Array,
    B_x: jax.Array,
    B_w_r: jax.Array,
    B_w_gate: jax.Array,
    B_w_up: jax.Array,
    B_w_down: jax.Array,
    c: jax.Array,
    w_mod: jax.Array,
):
    del B_x
    return _build(A_x, A_k_cache, A_v_cache, A_wq, A_wo, B_w_r, B_w_gate, B_w_up,
                  B_w_down, c, w_mod)
```

```python
import jax
import jax.numpy as jnp
import jax.experimental.pallas as pl
import jax.experimental.pallas.tpu as pltpu

_B, _D = 4, 512
_H, _DH = 32, 128
_EPS = 1e-5
_GRP = 4
_ROWS = 128
_WROWS = 32


def _layernorm(x):
    m = jnp.mean(x, axis=-1, keepdims=True)
    xc = x - m
    v = jnp.mean(xc * xc, axis=-1, keepdims=True)
    return xc / jnp.sqrt(v + _EPS)


def _dot(a, b):
    return jnp.dot(a, b, preferred_element_type=jnp.float32)


def _dot_nt(a, b):
    return jax.lax.dot_general(a, b, (((1,), (1,)), ((), ())),
                               preferred_element_type=jnp.float32)


def _loop(n, body):
    jax.lax.fori_loop(0, n, lambda t, carry: (body(t), carry)[1], 0)


def _kernel(x_hbm, c_hbm, wr_hbm, wmod_hbm, wq_hbm, wo_hbm, wg_hbm, wu_hbm, wd_hbm,
            k_hbm, v_hbm, o_ref,
            x_v, c_v, wr_v, wmod_v, wq_v, wo_v, wg_v, wu_v, wd_v, kbuf, vbuf, q_s,
            wsem, ksem, vsem):
    f32, bf16 = jnp.float32, jnp.bfloat16
    n_slabs = _B * _H
    sk = k_hbm.shape[0] // n_slabs
    ff = wg_hbm.shape[0]
    blk_rows = _GRP * sk
    streams = 2 * _GRP
    unit_chunks = sk // _ROWS
    rounds = unit_chunks // streams
    ahead = _GRP + 1
    first_last = n_slabs - _GRP
    S_X, S_C, S_WR, S_WMOD, S_WQ, S_WO, S_WG, S_WU, S_WD = range(9)

    def copy(src, dst, sem, queue):
        pltpu.make_async_copy(src, dst, sem).start(priority=queue)

    def wait_all(buf, sem):
        pltpu.make_async_copy(buf, buf, sem).wait()

    def copy_rows(src, dst, sem, chunk, rows, queue):
        sl = pl.ds(pl.multiple_of(chunk * rows, rows), rows)
        copy(src.at[sl], dst.at[sl], sem, queue)

    def kv_copy(u, off, slab):
        blk = u // _GRP
        slot = blk % 2
        off = pl.multiple_of(off, _ROWS)
        src = pl.ds(pl.multiple_of(blk * blk_rows + off, _ROWS), _ROWS)
        dst = pl.ds(off, _ROWS)
        copy(k_hbm.at[src], kbuf.at[slot, dst], ksem.at[slot, slab], 0)
        copy(v_hbm.at[src], vbuf.at[slot, dst], vsem.at[slot, slab], 1)

    def issue_unit(u):
        def body(t):
            for st in range(streams):
                kv_copy(u, st * (sk // 2) + ((u % _GRP) * rounds + t) * _ROWS, st // 2)
        _loop(rounds, body)

    def issue_unit_last(u):
        g = u % _GRP

        def body(t):
            for st in range(4):
                kv_copy(u, g * sk + st * (sk // 4) + t * _ROWS, g)
        _loop(unit_chunks // 4, body)

    nch = ff // _WROWS
    half = nch // 2

    def issue_ffn(lo, hi):
        if lo < min(hi, nch):
            def body(t):
                copy_rows(wg_hbm, wg_v, wsem.at[S_WG], lo + t, _WROWS, 0)
                copy_rows(wu_hbm, wu_v, wsem.at[S_WU], lo + t, _WROWS, 1)
            _loop(min(hi, nch) - lo, body)
        lo, hi = max(lo, nch) - nch, hi - nch
        if lo < min(hi, half):
            def body(t):
                copy_rows(wd_hbm, wd_v, wsem.at[S_WD], lo + t, _WROWS, 0)
                copy_rows(wd_hbm, wd_v, wsem.at[S_WD], half + lo + t, _WROWS, 1)
            _loop(min(hi, half) - lo, body)
        if hi > half and nch % 2:
            copy_rows(wd_hbm, wd_v, wsem.at[S_WD], nch - 1, _WROWS, 0)

    copy(c_hbm, c_v, wsem.at[S_C], 0)
    copy(x_hbm, x_v, wsem.at[S_X], 1)

    def start_wmod_wq(t):
        for st in range(4):
            r = pl.ds(pl.multiple_of((st * 16 + t) * 8, 8), 8)
            copy(wmod_hbm.at[r], wmod_v.at[r], wsem.at[S_WMOD], 0)
            for cols in (pl.ds(0, 2048), pl.ds(2048, 2048)):
                copy(wq_hbm.at[r, cols], wq_v.at[r, cols], wsem.at[S_WQ], 1)
    _loop(_D // 32, start_wmod_wq)
    copy(wr_hbm, wr_v, wsem.at[S_WR], 1)

    def start_wo(t):
        for st in range(4):
            copy_rows(wo_hbm, wo_v, wsem.at[S_WO], st * 32 + t, _WROWS, st % 2)
    _loop(_H * _DH // _WROWS // 4, start_wo)

    wait_all(c_v, wsem.at[S_C])
    wait_all(x_v, wsem.at[S_X])
    cc = c_v[...].astype(f32)
    sc = (cc * jax.nn.sigmoid(cc)).astype(bf16)
    x = x_v[...].astype(f32)
    ln_x = _layernorm(x)
    wait_all(wmod_v, wsem.at[S_WMOD])
    mod = _dot(sc, wmod_v[...])
    sa, ca, ga, sb, cb, gb = (mod[:, j * _D:(j + 1) * _D] for j in range(6))
    h = (ln_x * (1.0 + ca) + sa).astype(bf16)
    wait_all(wq_v, wsem.at[S_WQ])
    q = _dot(h, wq_v[...]).astype(bf16)
    for hh in range(_H):
        q_s[hh] = q[:, hh * _DH:(hh + 1) * _DH]

    _loop(ahead, issue_unit)
    wait_all(wo_v, wsem.at[S_WO])

    scale = _DH ** (-0.5)
    row = jax.lax.broadcasted_iota(jnp.int32, (_B, _DH), 0)
    n_ffn = nch + half + nch % 2
    ffn_pieces = (n_ffn // 4,) * 3 + (n_ffn - 3 * (n_ffn // 4), 0)

    def step(j, acc):
        slot, g = (j // _GRP) % 2, j % _GRP
        b, hh = j // _H, j % _H
        rs = pl.ds(pl.multiple_of(g * sk, sk), sk)
        wait_all(kbuf.at[slot, rs], ksem.at[slot, g])
        wait_all(vbuf.at[slot, rs], vsem.at[slot, g])
        s = _dot_nt(q_s[hh], kbuf[slot, rs, :]) * scale
        m = jnp.max(s, axis=-1, keepdims=True)
        p = jnp.exp(s - m)
        l = jnp.sum(p, axis=-1, keepdims=True)
        o = _dot(p.astype(bf16), vbuf[slot, rs, :]) / l
        o = jnp.where(row == b, o, 0.0).astype(bf16)
        acc = acc + _dot(o, wo_v[pl.ds(pl.multiple_of(hh * _DH, _DH), _DH), :])

        u = j + ahead
        pl.when(u < first_last)(lambda: issue_unit(u))
        pl.when((u >= first_last) & (u < n_slabs))(lambda: issue_unit_last(u))
        lo = 0
        for idx, cnt in enumerate(ffn_pieces):
            if cnt:
                pl.when(j == n_slabs - len(ffn_pieces) + idx)(
                    lambda lo=lo, cnt=cnt: issue_ffn(lo, lo + cnt))
            lo += cnt
        return acc

    attn = jax.lax.fori_loop(0, n_slabs, step, jnp.zeros((_B, _D), f32))

    x1 = x + ga * attn
    h2 = _layernorm(x1) * (1.0 + cb) + sb
    h2b = h2.astype(bf16)
    wait_all(wr_v, wsem.at[S_WR])
    wr = wr_v[...].astype(f32)
    r = sum(h2[:, j * 128:(j + 1) * 128] * wr[j:j + 1, :] for j in range(_D // 128))
    r = jnp.sum(r, axis=-1, keepdims=True)
    wait_all(wg_v, wsem.at[S_WG])
    gate = _dot_nt(h2b, wg_v[...])
    gate = gate * jax.nn.sigmoid(gate)
    wait_all(wu_v, wsem.at[S_WU])
    up = _dot_nt(h2b, wu_v[...])
    a = (gate * up).astype(bf16)
    wait_all(wd_v, wsem.at[S_WD])
    y = _dot(a, wd_v[...]) * jax.nn.sigmoid(r)
    upd = h2 * 0.0 + y
    o_ref[...] = (x1 + gb * (h2 + upd)).astype(o_ref.dtype)


@jax.jit
def pallas_adaLN_cond__gqa_block_cached__moe_arch_mod__decode_kernel(
    A_x: jax.Array,
    A_k_cache: jax.Array,
    A_v_cache: jax.Array,
    A_wq: jax.Array,
    A_wo: jax.Array,
    B_x: jax.Array,
    B_w_r: jax.Array,
    B_w_gate: jax.Array,
    B_w_up: jax.Array,
    B_w_down: jax.Array,
    c: jax.Array,
    w_mod: jax.Array,
):
    del B_x
    bf16 = jnp.bfloat16
    sk = A_k_cache.shape[2]
    ff = B_w_gate.shape[1]
    assert A_x.shape == (_B, 1, _D) and A_k_cache.shape == (_B, _H, sk, _DH)
    assert sk % (2 * _GRP * 2 * _ROWS) == 0 and sk % (4 * _ROWS) == 0 and ff % _WROWS == 0
    hbm = pl.BlockSpec(memory_space=pltpu.HBM)
    out = pl.pallas_call(
        _kernel,
        out_shape=jax.ShapeDtypeStruct((_B, _D), A_x.dtype),
        in_specs=[hbm] * 11,
        out_specs=pl.BlockSpec(memory_space=pltpu.VMEM),
        scratch_shapes=[
            pltpu.VMEM((_B, _D), bf16),
            pltpu.VMEM((_B, _D), bf16),
            pltpu.VMEM((_D // 128, 128), bf16),
            pltpu.VMEM((_D, 6 * _D), bf16),
            pltpu.VMEM((_D, _H * _DH), bf16),
            pltpu.VMEM((_H * _DH, _D), bf16),
            pltpu.VMEM((ff, _D), bf16),
            pltpu.VMEM((ff, _D), bf16),
            pltpu.VMEM((ff, _D), bf16),
            pltpu.VMEM((2, _GRP * sk, _DH), bf16),
            pltpu.VMEM((2, _GRP * sk, _DH), bf16),
            pltpu.VMEM((_H, _B, _DH), bf16),
            pltpu.SemaphoreType.DMA((9,)),
            pltpu.SemaphoreType.DMA((2, _GRP)),
            pltpu.SemaphoreType.DMA((2, _GRP)),
        ],
        compiler_params=pltpu.CompilerParams(vmem_limit_bytes=80 * 1024 * 1024),
        name="adaln_gqa_mod_decode",
    )(A_x.reshape(_B, _D), c, B_w_r.reshape(_D // 128, 128), w_mod, A_wq, A_wo,
      B_w_gate.T, B_w_up.T, B_w_down,
      A_k_cache.reshape(-1, _DH), A_v_cache.reshape(-1, _DH))
    return out.reshape(A_x.shape)
```

```python
import jax
import jax.numpy as jnp
import jax.experimental.pallas as pl
import jax.experimental.pallas.tpu as pltpu

_B, _D = 4, 512
_H, _DH = 32, 128
_EPS = 1e-5
_GRP = 4
_ROWS = 128
_WROWS = 32


def _layernorm(x):
    m = jnp.mean(x, axis=-1, keepdims=True)
    xc = x - m
    v = jnp.mean(xc * xc, axis=-1, keepdims=True)
    return xc / jnp.sqrt(v + _EPS)


def _dot(a, b):
    return jnp.dot(a, b, preferred_element_type=jnp.float32)


def _dot_nt(a, b):
    return jax.lax.dot_general(a, b, (((1,), (1,)), ((), ())),
                               preferred_element_type=jnp.float32)


def _loop(n, body):
    jax.lax.fori_loop(0, n, lambda t, carry: (body(t), carry)[1], 0)


def _kernel(x_hbm, c_hbm, wr_hbm, wmod_hbm, wq_hbm, wo_hbm, wg_hbm, wu_hbm, wd_hbm,
            k_hbm, v_hbm, o_ref,
            x_v, c_v, wr_v, wmod_v, wq_v, wo_v, wg_v, wu_v, wd_v, kbuf, vbuf, q_s,
            wsem, ksem, vsem):
    f32, bf16 = jnp.float32, jnp.bfloat16
    n_slabs = _B * _H
    sk = k_hbm.shape[0] // n_slabs
    ff = wg_hbm.shape[0]
    blk_rows = _GRP * sk
    streams = 2 * _GRP
    unit_chunks = sk // _ROWS
    rounds = unit_chunks // streams
    ahead = _GRP + 1
    first_last = n_slabs - _GRP
    S_X, S_C, S_WR, S_WMOD, S_WQ, S_WO, S_WG, S_WU, S_WD = range(9)

    def copy(src, dst, sem, queue):
        pltpu.make_async_copy(src, dst, sem).start(priority=queue)

    def wait_all(buf, sem):
        pltpu.make_async_copy(buf, buf, sem).wait()

    def copy_rows(src, dst, sem, chunk, rows, queue):
        sl = pl.ds(pl.multiple_of(chunk * rows, rows), rows)
        copy(src.at[sl], dst.at[sl], sem, queue)

    def kv_copy(u, off, slab):
        blk = u // _GRP
        slot = blk % 2
        off = pl.multiple_of(off, _ROWS)
        src = pl.ds(pl.multiple_of(blk * blk_rows + off, _ROWS), _ROWS)
        dst = pl.ds(off, _ROWS)
        copy(k_hbm.at[src], kbuf.at[slot, dst], ksem.at[slot, slab], 0)
        copy(v_hbm.at[src], vbuf.at[slot, dst], vsem.at[slot, slab], 1)

    def issue_unit(u):
        def body(t):
            for st in range(streams):
                kv_copy(u, st * (sk // 2) + ((u % _GRP) * rounds + t) * _ROWS, st // 2)
        _loop(rounds, body)

    def issue_unit_last(u):
        g = u % _GRP

        def body(t):
            for st in range(4):
                kv_copy(u, g * sk + st * (sk // 4) + t * _ROWS, g)
        _loop(unit_chunks // 4, body)

    nch = ff // _WROWS
    half = nch // 2

    def issue_ffn(lo, hi):
        if lo < min(hi, nch):
            def body(t):
                copy_rows(wg_hbm, wg_v, wsem.at[S_WG], lo + t, _WROWS, 0)
                copy_rows(wu_hbm, wu_v, wsem.at[S_WU], lo + t, _WROWS, 1)
            _loop(min(hi, nch) - lo, body)
        lo, hi = max(lo, nch) - nch, hi - nch
        if lo < min(hi, half):
            def body(t):
                copy_rows(wd_hbm, wd_v, wsem.at[S_WD], lo + t, _WROWS, 0)
                copy_rows(wd_hbm, wd_v, wsem.at[S_WD], half + lo + t, _WROWS, 1)
            _loop(min(hi, half) - lo, body)
        if hi > half and nch % 2:
            copy_rows(wd_hbm, wd_v, wsem.at[S_WD], nch - 1, _WROWS, 0)

    copy(c_hbm, c_v, wsem.at[S_C], 0)
    copy(x_hbm, x_v, wsem.at[S_X], 1)

    def start_wmod(t):
        for st in range(4):
            r = pl.ds(pl.multiple_of((st * 16 + t) * 8, 8), 8)
            copy(wmod_hbm.at[r], wmod_v.at[r], wsem.at[S_WMOD], st % 2)
    _loop(_D // 32, start_wmod)

    def start_wq(t):
        for hf in range(2):
            for st in range(4):
                r = pl.ds(pl.multiple_of((st * 16 + t) * 8, 8), 8)
                cols = pl.ds(hf * 2048, 2048)
                copy(wq_hbm.at[r, cols], wq_v.at[r, cols], wsem.at[S_WQ], st % 2)
    _loop(_D // 32, start_wq)
    copy(wr_hbm, wr_v, wsem.at[S_WR], 1)

    def start_wo(t):
        for st in range(4):
            copy_rows(wo_hbm, wo_v, wsem.at[S_WO], st * 32 + t, _WROWS, st % 2)
    _loop(_H * _DH // _WROWS // 4, start_wo)

    wait_all(c_v, wsem.at[S_C])
    wait_all(x_v, wsem.at[S_X])
    cc = c_v[...].astype(f32)
    sc = (cc * jax.nn.sigmoid(cc)).astype(bf16)
    x = x_v[...].astype(f32)
    ln_x = _layernorm(x)
    wait_all(wmod_v, wsem.at[S_WMOD])
    mod = _dot(sc, wmod_v[...])
    sa, ca, ga, sb, cb, gb = (mod[:, j * _D:(j + 1) * _D] for j in range(6))
    h = (ln_x * (1.0 + ca) + sa).astype(bf16)
    wait_all(wq_v, wsem.at[S_WQ])
    q = _dot(h, wq_v[...]).astype(bf16)
    for hh in range(_H):
        q_s[hh] = q[:, hh * _DH:(hh + 1) * _DH]

    _loop(ahead, issue_unit)
    wait_all(wo_v, wsem.at[S_WO])

    scale = _DH ** (-0.5)
    row = jax.lax.broadcasted_iota(jnp.int32, (_B, _DH), 0)
    n_ffn = nch + half + nch % 2
    ffn_pieces = (n_ffn // 4,) * 3 + (n_ffn - 3 * (n_ffn // 4), 0)

    def step(j, acc):
        slot, g = (j // _GRP) % 2, j % _GRP
        b, hh = j // _H, j % _H
        rs = pl.ds(pl.multiple_of(g * sk, sk), sk)
        wait_all(kbuf.at[slot, rs], ksem.at[slot, g])
        wait_all(vbuf.at[slot, rs], vsem.at[slot, g])
        s = _dot_nt(q_s[hh], kbuf[slot, rs, :]) * scale
        m = jnp.max(s, axis=-1, keepdims=True)
        p = jnp.exp(s - m)
        l = jnp.sum(p, axis=-1, keepdims=True)
        o = _dot(p.astype(bf16), vbuf[slot, rs, :]) / l
        o = jnp.where(row == b, o, 0.0).astype(bf16)
        acc = acc + _dot(o, wo_v[pl.ds(pl.multiple_of(hh * _DH, _DH), _DH), :])

        u = j + ahead
        pl.when(u < first_last)(lambda: issue_unit(u))
        pl.when((u >= first_last) & (u < n_slabs))(lambda: issue_unit_last(u))
        lo = 0
        for idx, cnt in enumerate(ffn_pieces):
            if cnt:
                pl.when(j == n_slabs - len(ffn_pieces) + idx)(
                    lambda lo=lo, cnt=cnt: issue_ffn(lo, lo + cnt))
            lo += cnt
        return acc

    attn = jax.lax.fori_loop(0, n_slabs, step, jnp.zeros((_B, _D), f32))

    x1 = x + ga * attn
    h2 = _layernorm(x1) * (1.0 + cb) + sb
    h2b = h2.astype(bf16)
    wait_all(wr_v, wsem.at[S_WR])
    wr = wr_v[...].astype(f32)
    r = sum(h2[:, j * 128:(j + 1) * 128] * wr[j:j + 1, :] for j in range(_D // 128))
    r = jnp.sum(r, axis=-1, keepdims=True)
    wait_all(wg_v, wsem.at[S_WG])
    gate = _dot_nt(h2b, wg_v[...])
    gate = gate * jax.nn.sigmoid(gate)
    wait_all(wu_v, wsem.at[S_WU])
    up = _dot_nt(h2b, wu_v[...])
    a = (gate * up).astype(bf16)
    wait_all(wd_v, wsem.at[S_WD])
    y = _dot(a, wd_v[...]) * jax.nn.sigmoid(r)
    upd = h2 * 0.0 + y
    o_ref[...] = (x1 + gb * (h2 + upd)).astype(o_ref.dtype)


@jax.jit
def pallas_adaLN_cond__gqa_block_cached__moe_arch_mod__decode_kernel(
    A_x: jax.Array,
    A_k_cache: jax.Array,
    A_v_cache: jax.Array,
    A_wq: jax.Array,
    A_wo: jax.Array,
    B_x: jax.Array,
    B_w_r: jax.Array,
    B_w_gate: jax.Array,
    B_w_up: jax.Array,
    B_w_down: jax.Array,
    c: jax.Array,
    w_mod: jax.Array,
):
    del B_x
    bf16 = jnp.bfloat16
    sk = A_k_cache.shape[2]
    ff = B_w_gate.shape[1]
    assert A_x.shape == (_B, 1, _D) and A_k_cache.shape == (_B, _H, sk, _DH)
    assert sk % (2 * _GRP * 2 * _ROWS) == 0 and sk % (4 * _ROWS) == 0 and ff % _WROWS == 0
    hbm = pl.BlockSpec(memory_space=pltpu.HBM)
    out = pl.pallas_call(
        _kernel,
        out_shape=jax.ShapeDtypeStruct((_B, _D), A_x.dtype),
        in_specs=[hbm] * 11,
        out_specs=pl.BlockSpec(memory_space=pltpu.VMEM),
        scratch_shapes=[
            pltpu.VMEM((_B, _D), bf16),
            pltpu.VMEM((_B, _D), bf16),
            pltpu.VMEM((_D // 128, 128), bf16),
            pltpu.VMEM((_D, 6 * _D), bf16),
            pltpu.VMEM((_D, _H * _DH), bf16),
            pltpu.VMEM((_H * _DH, _D), bf16),
            pltpu.VMEM((ff, _D), bf16),
            pltpu.VMEM((ff, _D), bf16),
            pltpu.VMEM((ff, _D), bf16),
            pltpu.VMEM((2, _GRP * sk, _DH), bf16),
            pltpu.VMEM((2, _GRP * sk, _DH), bf16),
            pltpu.VMEM((_H, _B, _DH), bf16),
            pltpu.SemaphoreType.DMA((9,)),
            pltpu.SemaphoreType.DMA((2, _GRP)),
            pltpu.SemaphoreType.DMA((2, _GRP)),
        ],
        compiler_params=pltpu.CompilerParams(vmem_limit_bytes=80 * 1024 * 1024),
        name="adaln_gqa_mod_decode",
    )(A_x.reshape(_B, _D), c, B_w_r.reshape(_D // 128, 128), w_mod, A_wq, A_wo,
      B_w_gate.T, B_w_up.T, B_w_down,
      A_k_cache.reshape(-1, _DH), A_v_cache.reshape(-1, _DH))
    return out.reshape(A_x.shape)
```
